```python
import jax
import jax.numpy as jnp

def _softmax(x, axis=-1):
    return jax.nn.softmax(x, axis=axis)

def _gelu(x):
    return jax.nn.gelu(x, approximate=True)

def _silu(x):
    return jax.nn.silu(x)

def _sigmoid(x):
    return jax.nn.sigmoid(x)

def _layernorm(x, axis=-1, eps=1e-05):
    m = jnp.mean(x, axis=axis, keepdims=True)
    v = jnp.var(x, axis=axis, keepdims=True)
    return (x - m) / jnp.sqrt(v + eps)

def _scatter_add(tgt, idx, src, axis=0):
    return tgt.at[idx].add(src)

def _segment_sum(src, seg, n):
    return jax.ops.segment_sum(src, seg, n)

class _Rng:

    def __init__(self, key):
        self._k = key

    def _next(self):
        self._k, sub = jax.random.split(self._k)
        return sub

    def normal(self, shape):
        return jax.random.normal(self._next(), shape, dtype=jnp.bfloat16)

    def randint(self, lo, hi, shape):
        return jax.random.randint(self._next(), shape, lo, hi, dtype=jnp.int32)

    def uniform(self, shape, lo=0.0, hi=1.0):
        return jax.random.uniform(self._next(), shape, jnp.bfloat16, lo, hi)

    def permutation(self, n):
        return jax.random.permutation(self._next(), n)
kernel_name = 'adaLN_cond__ssm_conv_h3__mixer_s_mlp__prompt'

def setup_inputs():
    _rng = _Rng(jax.random.key(int.from_bytes(__import__("os").urandom(4), "little")))
    _w = lambda a: (lambda t: t.astype(jnp.bfloat16) if jnp.issubdtype(t.dtype, jnp.floating) else t)(jnp.asarray(a))

    def _A_setup():
        B, S, D = (1, 2048, 640)
        ks = 4
        return {'q': _w((lambda *s: _rng.normal(s) * 0.05)(B, S, D)), 'k': _w((lambda *s: _rng.normal(s) * 0.05)(B, S, D)), 'v': _w((lambda *s: _rng.normal(s) * 0.05)(B, S, D)), 'shift_k': _w((lambda *s: _rng.normal(s) * 0.05)(D, ks) * 0.5), 'ssm_k': _w((lambda *s: _rng.normal(s) * 0.05)(D, S) * (1.0 / S ** 0.5)), 'ssm_D': _w((lambda *s: _rng.normal(s) * 0.05)(D))}
    _A_in = _A_setup()

    def _B_setup():
        B, S, D, F = (1, 2048, 640, 1728)
        return {'x': _w((lambda *s: _rng.normal(s) * 0.05)(B, S, D)), 'w1': _w((lambda *s: _rng.normal(s) * 0.05)(D, D) * D ** (-0.5)), 'w2': _w((lambda *s: _rng.normal(s) * 0.05)(D, D) * D ** (-0.5)), 'w3': _w((lambda *s: _rng.normal(s) * 0.05)(D, F) * D ** (-0.5)), 'w4': _w((lambda *s: _rng.normal(s) * 0.05)(F, D) * F ** (-0.5))}
    _B_in = _B_setup()
    return {'A_q': _A_in['q'], 'A_k': _A_in['k'], 'A_v': _A_in['v'], 'A_shift_k': _A_in['shift_k'], 'A_ssm_k': _A_in['ssm_k'], 'A_ssm_D': _A_in['ssm_D'], 'B_x': _B_in['x'], 'B_w1': _B_in['w1'], 'B_w2': _B_in['w2'], 'B_w3': _B_in['w3'], 'B_w4': _B_in['w4'], 'c': _w((lambda *s: _rng.normal(s) * 0.05)(1, 640)), 'w_mod': _w((lambda *s: _rng.normal(s) * 0.05)(640, 6 * 640) * 640 ** (-0.5))}

def reference(A_q, A_k, A_v, A_shift_k, A_ssm_k, A_ssm_D, B_x, B_w1, B_w2, B_w3, B_w4, c, w_mod):

    def _A_ref(q, k, v, shift_k, ssm_k, ssm_D):
        B, S, D = q.shape
        ks = shift_k.shape[-1]
        k_pad = jnp.pad(k, ((0, 0), (ks - 1, 0), (0, 0)))
        k_shift = jnp.zeros_like(k)
        for t in range(ks):
            k_shift = k_shift + k_pad[:, t:t + S, :] * shift_k[:, ks - 1 - t][None, None, :]
        kv = k_shift * v
        L = 2 * S
        kv_pad = jnp.pad(kv, ((0, 0), (0, S), (0, 0)))
        kf_pad = jnp.pad(ssm_k, ((0, 0), (0, S)))
        kv_f = (lambda x, axes=(-2, -1): jnp.fft.rfft2(x.astype(jnp.float32), axes=axes))(kv_pad[:, None, :, :], axes=(1, 2))
        kf_f = (lambda x, axes=(-2, -1): jnp.fft.rfft2(x.astype(jnp.float32), axes=axes))(kf_pad[:, None, :], axes=(1, 2))
        kf_f = (lambda x, *d: x.transpose(*d))(kf_f, 1, 2, 0)
        y_f = kv_f * kf_f[None, :, :, :]
        y = (lambda x, s, axes=(-2, -1): jnp.fft.irfft2(x, s=s, axes=axes).astype(jnp.bfloat16))(y_f, (1, L), axes=(1, 2))[:, 0, :S, :]
        y = y + kv * ssm_D[None, None, :]
        return q * y

    def _B_ref(x, w1, w2, w3, w4):
        B, S, D = x.shape
        h = _gelu(_layernorm(x, axis=-1) @ w1)
        c = D // 4
        g0 = jnp.pad(h[:, :, 0 * c:1 * c], ((0, 0), (1, 0), (0, 0)))[:, :S, :]
        g1 = jnp.pad(h[:, :, 1 * c:2 * c], ((0, 0), (0, 1), (0, 0)))[:, 1:, :]
        g2 = jnp.pad(h[:, :, 2 * c:3 * c], ((0, 0), (2, 0), (0, 0)))[:, :S, :]
        g3 = jnp.pad(h[:, :, 3 * c:], ((0, 0), (0, 2), (0, 0)))[:, 2:, :]
        hs = jnp.concatenate([g0, g1, g2, g3], axis=-1) @ w2
        x1 = x + hs
        h2 = _gelu(_layernorm(x1, axis=-1) @ w3) @ w4
        return x1 + h2
    x = A_q
    mod = (_silu(c) @ w_mod).reshape(c.shape[0], 6, 1, -1)
    sa, ca, ga, sb, cb, gb = (mod[:, 0].copy(), mod[:, 1].copy(), mod[:, 2].copy(), mod[:, 3].copy(), mod[:, 4].copy(), mod[:, 5].copy())
    h = _layernorm(x, axis=-1) * (1 + ca) + sa
    x = x + ga * _A_ref(h, A_k, A_v, A_shift_k, A_ssm_k, A_ssm_D)
    h = _layernorm(x, axis=-1) * (1 + cb) + sb
    x = x + gb * _B_ref(h, B_w1, B_w2, B_w3, B_w4)
    return x
```

```python
import jax
import jax.numpy as jnp
import numpy as np
import jax.experimental.pallas as pl
import jax.experimental.pallas.tpu as pltpu

S, D, FF = 2048, 640, 1728
T = 128
NB = S // T
NL = D // 128
CH = 256
NC = S // CH
AB = 4
F32, BF16 = jnp.float32, jnp.bfloat16

_theta = (np.pi / 2 + 2 * np.pi * np.arange(T)) / T
_ang = _theta[:, None] * np.arange(T)[None, :]
_FWD = np.concatenate([np.cos(_ang), np.sin(_ang)], 0).astype(np.float32)
_INV = np.ascontiguousarray(_FWD.T) / T


def _dot(a, b):
    return jnp.dot(a, b, preferred_element_type=F32)


def _ln(x):
    m = jnp.mean(x, axis=-1, keepdims=True)
    d = x - m
    v = jnp.mean(d * d, axis=-1, keepdims=True)
    return d * jax.lax.rsqrt(v + 1e-5)


def _gelu(x):
    c0 = float(np.sqrt(2 / np.pi))
    c1 = c0 * 0.044715
    hx = 0.5 * x
    return hx + hx * jnp.tanh(x * (c0 + c1 * (x * x)))


def _kernel(q_h, k_h, v_h, sk_ref, fk_h, sd_ref, w1_h, w2_h, w3_h, w4_h, c_ref,
            wm_h, fwd_ref, inv_ref, o_h,
            q_v, k_v, v_v, fk_v, w1_v, w2_v, w3_v, w4_v, wm_v, o_v,
            kpad, kv_s, xf, kf, yf, hh, xs, h1s, sems, osems):
    copies = [pltpu.make_async_copy(h, v, sems.at[i]) for i, (h, v) in enumerate(
        [(fk_h, fk_v), (k_h, k_v), (v_h, v_v), (wm_h, wm_v), (q_h, q_v),
         (w1_h, w1_v), (w2_h, w2_v), (w3_h, w3_v), (w4_h, w4_v)])]
    for cp in copies:
        cp.start()
    cp_fk, cp_k, cp_v, cp_wm, cp_q, cp_w1, cp_w2, cp_w3, cp_w4 = copies
    fwd = fwd_ref[...]

    cp_fk.wait()
    for j in range(NB):
        kj = jax.lax.dot_general(fwd, fk_v[:, j * T:(j + 1) * T],
                                 (((1,), (1,)), ((), ())),
                                 preferred_element_type=F32)
        if j == 0:
            cur = kj
        else:
            cur = jnp.concatenate([kj[:T] + prev[T:], kj[T:] - prev[:T]], 0)
        prev = kj
        for l in range(NL):
            kf[l, j] = cur[:, l * 128:(l + 1) * 128]

    cp_k.wait()
    kpad[0:8, :] = jnp.zeros((8, D), F32)

    @pl.loop(0, NB)
    def _(b):
        r = pl.multiple_of(b * T, T)
        kpad[pl.ds(pl.multiple_of(r + 8, 8), T), :] = k_v[pl.ds(r, T), :].astype(F32)

    cp_v.wait()

    @pl.loop(0, NB)
    def _(b):
        r = pl.multiple_of(b * T, T)
        win = kpad[pl.ds(r, T + 8), :]
        ks = win[8:] * sk_ref[0:1, :]
        for j in range(1, 4):
            ks = ks + win[8 - j:8 - j + T] * sk_ref[j:j + 1, :]
        kv = ks * v_v[pl.ds(r, T), :].astype(F32)
        kv_s[pl.ds(r, T), :] = kv
        xb = _dot(fwd, kv.astype(BF16))
        for l in range(NL):
            xf[l, b] = xb[:, l * 128:(l + 1) * 128]

    @pl.loop(0, NL * 8)
    def _(i):
        l = i // 8
        f0 = pl.multiple_of((i % 8) * 16, 16)
        re, im = pl.ds(f0, 16), pl.ds(pl.multiple_of(f0 + T, 16), 16)
        for a0 in range(0, NB, AB):
            yr, yi = [None] * AB, [None] * AB
            win = {}
            for b in range(a0 + AB):
                xr, xi = xf[l, b, re, :], xf[l, b, im, :]
                for a in range(max(a0, b), a0 + AB):
                    if a - b not in win:
                        win[a - b] = (kf[l, a - b, re, :], kf[l, a - b, im, :])
                    kr, ki = win[a - b]
                    pr, pi = xr * kr - xi * ki, xr * ki + xi * kr
                    n = a - a0
                    yr[n] = pr if yr[n] is None else yr[n] + pr
                    yi[n] = pi if yi[n] is None else yi[n] + pi
            for n in range(AB):
                yf[l, a0 + n, re, :] = yr[n].astype(BF16)
                yf[l, a0 + n, im, :] = yi[n].astype(BF16)

    cp_wm.wait()
    c = c_ref[...].astype(F32)
    sc = (c * jax.nn.sigmoid(c)).astype(BF16)
    mod = _dot(jnp.broadcast_to(sc, (16, D)), wm_v[...])[0:1, :]
    sa, ca, ga, sb, cb, gb = [mod[:, n * D:(n + 1) * D] for n in range(6)]
    ca1, cb1 = 1.0 + ca, 1.0 + cb
    sd = sd_ref[...].astype(F32)
    inv = inv_ref[...]

    cp_q.wait()
    cp_w1.wait()
    hh[0:8, :] = jnp.zeros((8, D), F32)
    hh[S + 8:S + 16, :] = jnp.zeros((8, D), F32)

    def stage_a(ci):
        r = pl.multiple_of(ci * CH, CH)
        rows = pl.ds(r, CH)
        y = jnp.concatenate(
            [jnp.concatenate([_dot(inv, yf[l, ci * (CH // T) + n]) for l in range(NL)], 1)
             for n in range(CH // T)], 0)
        y = y + kv_s[rows, :] * sd
        q = q_v[rows, :].astype(F32)
        x = q + ga * ((_ln(q) * ca1 + sa) * y)
        h1 = _ln(x) * cb1 + sb
        xs[rows, :] = x
        h1s[rows, :] = h1
        hh[pl.ds(pl.multiple_of(r + 8, 8), CH), :] = _gelu(
            _dot(_ln(h1).astype(BF16), w1_v[...]))

    def out_copy(ci):
        rows = pl.ds(pl.multiple_of(ci * CH, CH), CH)
        return pltpu.make_async_copy(o_v.at[rows, :], o_h.at[rows, :], osems.at[ci])

    def stage_b(ci):
        r = pl.multiple_of(ci * CH, CH)
        rows = pl.ds(r, CH)
        lane = jax.lax.broadcasted_iota(jnp.int32, (CH, 128), 1)
        shifts = (-1, 1, -2, 2)
        parts = []
        for l in range(NL):
            win = hh[pl.ds(r, CH + 16), l * 128:(l + 1) * 128]
            g_lo, g_hi = (l * 128) // 160, (l * 128 + 127) // 160
            p = win[8 + shifts[g_lo]:8 + shifts[g_lo] + CH]
            if g_hi != g_lo:
                p2 = win[8 + shifts[g_hi]:8 + shifts[g_hi] + CH]
                p = jnp.where(lane < g_hi * 160 - l * 128, p, p2)
            parts.append(p.astype(BF16))
        x1 = h1s[rows, :] + _dot(jnp.concatenate(parts, 1), w2_v[...])
        g = _gelu(_dot(_ln(x1).astype(BF16), w3_v[...])).astype(BF16)
        res = x1 + _dot(g, w4_v[...])
        o_v[rows, :] = (xs[rows, :] + gb * res).astype(BF16)
        out_copy(ci).start()

    stage_a(0)
    cp_w2.wait()
    cp_w3.wait()
    cp_w4.wait()

    @pl.loop(0, NC - 1)
    def _(ci):
        stage_a(ci + 1)
        stage_b(ci)

    stage_b(NC - 1)
    for ci in range(NC):
        out_copy(ci).wait()


@jax.jit
def pallas_adaLN_cond__ssm_conv_h3__mixer_s_mlp__prompt_kernel(
    A_q, A_k, A_v, A_shift_k, A_ssm_k, A_ssm_D, B_x, B_w1, B_w2, B_w3, B_w4, c, w_mod,
):
    hbm = pl.BlockSpec(memory_space=pl.ANY)
    vm = pl.BlockSpec(memory_space=pltpu.VMEM)
    V = pltpu.VMEM
    out = pl.pallas_call(
        _kernel,
        out_shape=jax.ShapeDtypeStruct((S, D), BF16),
        in_specs=[hbm, hbm, hbm, vm, hbm, vm, hbm, hbm, hbm, hbm, vm, hbm, vm, vm],
        out_specs=hbm,
        scratch_shapes=[
            V((S, D), BF16), V((S, D), BF16), V((S, D), BF16), V((D, S), BF16),
            V((D, D), BF16), V((D, D), BF16), V((D, FF), BF16), V((FF, D), BF16),
            V((D, 6 * D), BF16), V((S, D), BF16),
            V((S + 8, D), F32), V((S, D), F32),
            V((NL, NB, 2 * T, 128), F32), V((NL, NB, 2 * T, 128), F32),
            V((NL, NB, 2 * T, 128), BF16),
            V((S + 16, D), F32), V((S, D), F32), V((S, D), F32),
            pltpu.SemaphoreType.DMA((9,)), pltpu.SemaphoreType.DMA((NC,)),
        ],
        compiler_params=pltpu.CompilerParams(vmem_limit_bytes=110 * 1024 * 1024),
    )(A_q[0], A_k[0], A_v[0], A_shift_k.T.astype(F32), A_ssm_k, A_ssm_D.reshape(1, D),
      B_w1, B_w2, B_w3, B_w4, c, w_mod,
      jnp.asarray(_FWD, BF16), jnp.asarray(_INV, BF16))
    return out[None]
```

```python
import jax
import jax.numpy as jnp
import numpy as np
import jax.experimental.pallas as pl
import jax.experimental.pallas.tpu as pltpu

S, D, FF = 2048, 640, 1728
T = 128
NB = S // T
NL = D // 128
CH = 256
NC = S // CH
AB = 4
F32, BF16 = jnp.float32, jnp.bfloat16

_theta = (np.pi / 2 + 2 * np.pi * np.arange(T)) / T
_ang = _theta[:, None] * np.arange(T)[None, :]
_FWD = np.concatenate([np.cos(_ang), np.sin(_ang)], 0).astype(np.float32)
_INV = np.ascontiguousarray(_FWD.T) / T


def _dot(a, b):
    return jnp.dot(a, b, preferred_element_type=F32)


def _dot_nt(a, b):
    return jax.lax.dot_general(a, b, (((1,), (1,)), ((), ())), preferred_element_type=F32)


def _ln(x):
    m = jnp.mean(x, axis=-1, keepdims=True)
    d = x - m
    v = jnp.mean(d * d, axis=-1, keepdims=True)
    return d * jax.lax.rsqrt(v + 1e-5)


def _gelu(x):
    c0 = float(np.sqrt(2 / np.pi))
    c1 = c0 * 0.044715
    hx = 0.5 * x
    return hx + hx * jnp.tanh(x * (c0 + c1 * (x * x)))


def _kernel(q_h, k_h, v_h, sk_h, fk_h, sd_h, w1_h, w2_h, w3_h, w4_h, c_h,
            wm_h, fwd_h, inv_h, o_h,
            sk_v, sd_ref, c_ref, fwd_ref, inv_ref,
            q_v, k_v, v_v, fk_v, w1_v, w2_v, w3_v, w4_v, wm_v, o_v,
            kpad, kv_s, xf, kf, yf, hh, xs, h1s, sems, osems):
    copies = [pltpu.make_async_copy(h, v, sems.at[i]) for i, (h, v) in enumerate(
        [(fwd_h, fwd_ref), (sk_h, sk_v), (sd_h, sd_ref), (c_h, c_ref), (inv_h, inv_ref),
         (fk_h, fk_v), (k_h, k_v), (v_h, v_v), (wm_h, wm_v), (q_h, q_v),
         (w1_h, w1_v), (w2_h, w2_v), (w3_h, w3_v), (w4_h, w4_v)])]
    for cp in copies[:6]:
        cp.start()
    cp_fk, cp_k, cp_v, cp_wm, cp_q, cp_w1, cp_w2, cp_w3, cp_w4 = copies[5:]
    for cp in copies[:5]:
        cp.wait()
    sk = sk_v[...].astype(F32)
    fwd = fwd_ref[...]

    cp_fk.wait()
    cp_k.start()
    cp_v.start()
    xs[0:2 * T, :] = jnp.zeros((2 * T, D), F32)

    @pl.loop(0, NB, step=2)
    def _(j0):
        prev = xs[0:2 * T, :]
        for j in (j0, j0 + 1):
            kj = _dot_nt(fwd, fk_v[:, pl.ds(pl.multiple_of(j * T, T), T)])
            cur = jnp.concatenate([kj[:T] + prev[T:], kj[T:] - prev[:T]], 0)
            prev = kj
            for l in range(NL):
                kf[l, j] = cur[:, l * 128:(l + 1) * 128]
        xs[0:2 * T, :] = prev

    cp_k.wait()
    kpad[0:8, :] = jnp.zeros((8, D), F32)

    @pl.loop(0, NB)
    def _(b):
        r = pl.multiple_of(b * T, T)
        kpad[pl.ds(pl.multiple_of(r + 8, 8), T), :] = k_v[pl.ds(r, T), :].astype(F32)

    cp_v.wait()
    for cp in copies[8:]:
        cp.start()

    @pl.loop(0, NB, unroll=2)
    def _(b):
        r = pl.multiple_of(b * T, T)
        win = kpad[pl.ds(r, T + 8), :]
        ks = win[8:] * sk[0:1, :]
        for j in range(1, 4):
            ks = ks + win[8 - j:8 - j + T] * sk[j:j + 1, :]
        kv = ks * v_v[pl.ds(r, T), :].astype(F32)
        kv_s[pl.ds(r, T), :] = kv
        xb = _dot(fwd, kv.astype(BF16))
        for l in range(NL):
            xf[l, b] = xb[:, l * 128:(l + 1) * 128]

    @pl.loop(0, NL * 8)
    def _(i):
        l = i // 8
        f0 = pl.multiple_of((i % 8) * 16, 16)
        re, im = pl.ds(f0, 16), pl.ds(pl.multiple_of(f0 + T, 16), 16)
        for a0 in range(0, NB, AB):
            yr, yi = [None] * AB, [None] * AB
            win = {}
            for b in range(a0 + AB):
                xr, xi = xf[l, b, re, :], xf[l, b, im, :]
                for a in range(max(a0, b), a0 + AB):
                    if a - b not in win:
                        win[a - b] = (kf[l, a - b, re, :], kf[l, a - b, im, :])
                    kr, ki = win[a - b]
                    pr, pi = xr * kr - xi * ki, xr * ki + xi * kr
                    n = a - a0
                    yr[n] = pr if yr[n] is None else yr[n] + pr
                    yi[n] = pi if yi[n] is None else yi[n] + pi
            for n in range(AB):
                yf[l, a0 + n, re, :] = yr[n].astype(BF16)
                yf[l, a0 + n, im, :] = yi[n].astype(BF16)

    cp_wm.wait()
    c = c_ref[...].astype(F32)
    sc = (c * jax.nn.sigmoid(c)).astype(BF16)
    mod = _dot(jnp.broadcast_to(sc, (16, D)), wm_v[...])[0:1, :]
    sa, ca, ga, sb, cb, gb = [mod[:, n * D:(n + 1) * D] for n in range(6)]
    ca1, cb1 = 1.0 + ca, 1.0 + cb
    sd = sd_ref[...].astype(F32)
    inv = inv_ref[...]

    cp_q.wait()
    cp_w1.wait()
    hh[0:8, :] = jnp.zeros((8, D), F32)
    hh[S + 8:S + 16, :] = jnp.zeros((8, D), F32)

    def stage_a(ci):
        r = pl.multiple_of(ci * CH, CH)
        rows = pl.ds(r, CH)
        y = jnp.concatenate(
            [jnp.concatenate([_dot(inv, yf[l, ci * (CH // T) + n]) for l in range(NL)], 1)
             for n in range(CH // T)], 0)
        y = y + kv_s[rows, :] * sd
        q = q_v[rows, :].astype(F32)
        x = q + ga * ((_ln(q) * ca1 + sa) * y)
        h1 = _ln(x) * cb1 + sb
        xs[rows, :] = x
        h1s[rows, :] = h1
        hh[pl.ds(pl.multiple_of(r + 8, 8), CH), :] = _gelu(
            _dot(_ln(h1).astype(BF16), w1_v[...]))

    def out_copy(ci):
        rows = pl.ds(pl.multiple_of(ci * CH, CH), CH)
        return pltpu.make_async_copy(o_v.at[rows, :], o_h.at[rows, :], osems.at[ci])

    def stage_b(ci):
        r = pl.multiple_of(ci * CH, CH)
        rows = pl.ds(r, CH)
        lane = jax.lax.broadcasted_iota(jnp.int32, (CH, 128), 1)
        shifts = (-1, 1, -2, 2)
        parts = []
        for l in range(NL):
            win = hh[pl.ds(r, CH + 16), l * 128:(l + 1) * 128]
            g_lo, g_hi = (l * 128) // 160, (l * 128 + 127) // 160
            p = win[8 + shifts[g_lo]:8 + shifts[g_lo] + CH]
            if g_hi != g_lo:
                p2 = win[8 + shifts[g_hi]:8 + shifts[g_hi] + CH]
                p = jnp.where(lane < g_hi * 160 - l * 128, p, p2)
            parts.append(p.astype(BF16))
        x1 = h1s[rows, :] + _dot(jnp.concatenate(parts, 1), w2_v[...])
        u = _ln(x1).astype(BF16)
        gs, outs = [], []
        for n0 in range(0, FF, 256):
            gs.append(_gelu(_dot_nt(u, w3_v[n0:min(n0 + 256, FF), :])).astype(BF16))
        g = jnp.concatenate(gs, 1)
        for n0 in range(0, D, 128):
            outs.append(_dot(g, w4_v[:, n0:n0 + 128]))
        res = x1 + jnp.concatenate(outs, 1)
        o_v[rows, :] = (xs[rows, :] + gb * res).astype(BF16)
        out_copy(ci).start()

    for cp in (cp_w2, cp_w3, cp_w4):
        cp.wait()

    @pl.loop(0, NC + 1)
    def _(ci):
        pl.when(ci < NC)(lambda: stage_a(ci))
        pl.when(ci > 0)(lambda: stage_b(ci - 1))

    for ci in range(NC):
        out_copy(ci).wait()


@jax.jit
def pallas_adaLN_cond__ssm_conv_h3__mixer_s_mlp__prompt_kernel(
    A_q, A_k, A_v, A_shift_k, A_ssm_k, A_ssm_D, B_x, B_w1, B_w2, B_w3, B_w4, c, w_mod,
):
    hbm = pl.BlockSpec(memory_space=pltpu.HBM)
    V = pltpu.VMEM
    out = pl.pallas_call(
        _kernel,
        out_shape=jax.ShapeDtypeStruct((S, D), BF16),
        in_specs=[hbm] * 14,
        out_specs=hbm,
        scratch_shapes=[
            V((4, D), BF16), V((1, D), BF16), V((1, D), BF16),
            V((2 * T, T), BF16), V((T, 2 * T), BF16),
            V((S, D), BF16), V((S, D), BF16), V((S, D), BF16), V((D, S), BF16),
            V((D, D), BF16), V((D, D), BF16), V((FF, D), BF16), V((FF, D), BF16),
            V((D, 6 * D), BF16), V((S, D), BF16),
            V((S + 8, D), F32), V((S, D), F32),
            V((NL, NB, 2 * T, 128), F32), V((NL, NB, 2 * T, 128), F32),
            V((NL, NB, 2 * T, 128), BF16),
            V((S + 16, D), F32), V((S, D), F32), V((S, D), F32),
            pltpu.SemaphoreType.DMA((14,)), pltpu.SemaphoreType.DMA((NC,)),
        ],
        compiler_params=pltpu.CompilerParams(vmem_limit_bytes=110 * 1024 * 1024),
    )(A_q[0], A_k[0], A_v[0], A_shift_k.T, A_ssm_k, A_ssm_D.reshape(1, D),
      B_w1, B_w2, B_w3.T, B_w4, c, w_mod,
      jnp.asarray(_FWD, BF16), jnp.asarray(_INV, BF16))
    return out[None]
```

```python
import jax
import jax.numpy as jnp
import numpy as np
import jax.experimental.pallas as pl
import jax.experimental.pallas.tpu as pltpu

S, D, FF = 2048, 640, 1728
T = 128
NB = S // T
NL = D // 128
CH = 512
NC = S // CH
AB = 2
F32, BF16 = jnp.float32, jnp.bfloat16

_theta = (np.pi / 2 + 2 * np.pi * np.arange(T)) / T
_ang = _theta[:, None] * np.arange(T)[None, :]
_FWD = np.concatenate([np.cos(_ang), np.sin(_ang)], 0).astype(np.float32)
_INV = np.ascontiguousarray(_FWD.T) / T


def _dot(a, b):
    return jnp.dot(a, b, preferred_element_type=F32)


def _dot_nt(a, b):
    return jax.lax.dot_general(a, b, (((1,), (1,)), ((), ())), preferred_element_type=F32)


def _ln(x):
    m = jnp.mean(x, axis=-1, keepdims=True)
    d = x - m
    v = jnp.mean(d * d, axis=-1, keepdims=True)
    return d * jax.lax.rsqrt(v + 1e-5)


def _gelu(x):
    c0 = float(np.sqrt(2 / np.pi))
    c1 = c0 * 0.044715
    hx = 0.5 * x
    return hx + hx * jnp.tanh(x * (c0 + c1 * (x * x)))


def _kernel(q_h, k_h, v_h, sk_h, fk_h, sd_h, w1_h, w2_h, w3_h, w4_h, c_h,
            wm_h, fwd_h, inv_h, o_h,
            sk_v, sd_ref, c_ref, fwd_ref, inv_ref,
            q_v, k_v, v_v, fk_v, w1_v, w2_v, w3_v, w4_v, wm_v, o_v,
            kpad, kv_s, xf, kf, yf, hh, xs, h1s, sems, osems):
    copies = [pltpu.make_async_copy(h, v, sems.at[i]) for i, (h, v) in enumerate(
        [(fwd_h, fwd_ref), (sk_h, sk_v), (sd_h, sd_ref), (c_h, c_ref), (inv_h, inv_ref),
         (fk_h, fk_v), (k_h, k_v), (v_h, v_v), (wm_h, wm_v), (q_h, q_v),
         (w1_h, w1_v), (w2_h, w2_v), (w3_h, w3_v), (w4_h, w4_v)])]
    for cp in copies[:6]:
        cp.start()
    cp_fk, cp_k, cp_v, cp_wm, cp_q, cp_w1, cp_w2, cp_w3, cp_w4 = copies[5:]
    for cp in copies[:5]:
        cp.wait()
    sk = sk_v[...].astype(F32)
    fwd = fwd_ref[...]

    cp_fk.wait()
    cp_k.start()
    cp_v.start()
    xs[0:2 * T, :] = jnp.zeros((2 * T, D), F32)

    @pl.loop(0, NB, step=4)
    def _(j0):
        prev = xs[0:2 * T, :]
        for j in (j0, j0 + 1, j0 + 2, j0 + 3):
            kj = _dot_nt(fwd, fk_v[:, pl.ds(pl.multiple_of(j * T, T), T)])
            cur = jnp.concatenate([kj[:T] + prev[T:], kj[T:] - prev[:T]], 0)
            prev = kj
            for l in range(NL):
                kf[l, j] = cur[:, l * 128:(l + 1) * 128]
        xs[0:2 * T, :] = prev

    cp_k.wait()
    kpad[0:8, :] = jnp.zeros((8, D), F32)

    @pl.loop(0, NB)
    def _(b):
        r = pl.multiple_of(b * T, T)
        kpad[pl.ds(pl.multiple_of(r + 8, 8), T), :] = k_v[pl.ds(r, T), :].astype(F32)

    cp_v.wait()
    for cp in copies[8:]:
        cp.start()

    @pl.loop(0, NB, unroll=2)
    def _(b):
        r = pl.multiple_of(b * T, T)
        win = kpad[pl.ds(r, T + 8), :]
        ks = win[8:] * sk[0:1, :]
        for j in range(1, 4):
            ks = ks + win[8 - j:8 - j + T] * sk[j:j + 1, :]
        kv = ks * v_v[pl.ds(r, T), :].astype(F32)
        kv_s[pl.ds(r, T), :] = kv
        xb = _dot(fwd, kv.astype(BF16))
        for l in range(NL):
            xf[l, b] = xb[:, l * 128:(l + 1) * 128]

    @pl.loop(0, NL * 8)
    def _(i):
        l = i // 8
        f0 = pl.multiple_of((i % 8) * 16, 16)
        re, im = pl.ds(f0, 16), pl.ds(pl.multiple_of(f0 + T, 16), 16)
        for a0 in range(0, NB, AB):
            yr, yi = [None] * AB, [None] * AB
            win = {}
            for b in range(a0 + AB):
                xr, xi = xf[l, b, re, :], xf[l, b, im, :]
                for a in range(max(a0, b), a0 + AB):
                    if a - b not in win:
                        win[a - b] = (kf[l, a - b, re, :], kf[l, a - b, im, :])
                    kr, ki = win[a - b]
                    pr, pi = xr * kr - xi * ki, xr * ki + xi * kr
                    n = a - a0
                    yr[n] = pr if yr[n] is None else yr[n] + pr
                    yi[n] = pi if yi[n] is None else yi[n] + pi
            for n in range(AB):
                yf[l, a0 + n, re, :] = yr[n].astype(BF16)
                yf[l, a0 + n, im, :] = yi[n].astype(BF16)

    cp_wm.wait()
    c = c_ref[...].astype(F32)
    sc = (c * jax.nn.sigmoid(c)).astype(BF16)
    mod = _dot(jnp.broadcast_to(sc, (16, D)), wm_v[...])[0:1, :]
    sa, ca, ga, sb, cb, gb = [mod[:, n * D:(n + 1) * D] for n in range(6)]
    ca1, cb1 = 1.0 + ca, 1.0 + cb
    sd = sd_ref[...].astype(F32)
    inv = inv_ref[...]

    cp_q.wait()
    cp_w1.wait()
    hh[0:8, :] = jnp.zeros((8, D), F32)
    hh[S + 8:S + 16, :] = jnp.zeros((8, D), F32)

    def stage_a(ci):
        r = pl.multiple_of(ci * CH, CH)
        rows = pl.ds(r, CH)
        y = jnp.concatenate(
            [jnp.concatenate([_dot(inv, yf[l, ci * (CH // T) + n]) for l in range(NL)], 1)
             for n in range(CH // T)], 0)
        y = y + kv_s[rows, :] * sd
        q = q_v[rows, :].astype(F32)
        x = q + ga * ((_ln(q) * ca1 + sa) * y)
        h1 = _ln(x) * cb1 + sb
        xs[rows, :] = x
        h1s[rows, :] = h1
        hh[pl.ds(pl.multiple_of(r + 8, 8), CH), :] = _gelu(
            _dot(_ln(h1).astype(BF16), w1_v[...]))

    def out_copy(ci):
        rows = pl.ds(pl.multiple_of(ci * CH, CH), CH)
        return pltpu.make_async_copy(o_v.at[rows, :], o_h.at[rows, :], osems.at[ci])

    def stage_b(ci):
        r = pl.multiple_of(ci * CH, CH)
        rows = pl.ds(r, CH)
        lane = jax.lax.broadcasted_iota(jnp.int32, (CH, 128), 1)
        shifts = (-1, 1, -2, 2)
        parts = []
        for l in range(NL):
            win = hh[pl.ds(r, CH + 16), l * 128:(l + 1) * 128]
            g_lo, g_hi = (l * 128) // 160, (l * 128 + 127) // 160
            p = win[8 + shifts[g_lo]:8 + shifts[g_lo] + CH]
            if g_hi != g_lo:
                p2 = win[8 + shifts[g_hi]:8 + shifts[g_hi] + CH]
                p = jnp.where(lane < g_hi * 160 - l * 128, p, p2)
            parts.append(p.astype(BF16))
        x1 = h1s[rows, :] + _dot(jnp.concatenate(parts, 1), w2_v[...])
        u = _ln(x1).astype(BF16)
        gs, outs = [], []
        for n0 in range(0, FF, 256):
            gs.append(_gelu(_dot_nt(u, w3_v[n0:min(n0 + 256, FF), :])).astype(BF16))
        g = jnp.concatenate(gs, 1)
        for n0 in range(0, D, 128):
            outs.append(_dot(g, w4_v[:, n0:n0 + 128]))
        res = x1 + jnp.concatenate(outs, 1)
        o_v[rows, :] = (xs[rows, :] + gb * res).astype(BF16)
        out_copy(ci).start()

    for cp in (cp_w2, cp_w3, cp_w4):
        cp.wait()

    @pl.loop(0, NC + 1)
    def _(ci):
        pl.when(ci < NC)(lambda: stage_a(ci))
        pl.when(ci > 0)(lambda: stage_b(ci - 1))

    for ci in range(NC):
        out_copy(ci).wait()


@jax.jit
def pallas_adaLN_cond__ssm_conv_h3__mixer_s_mlp__prompt_kernel(
    A_q, A_k, A_v, A_shift_k, A_ssm_k, A_ssm_D, B_x, B_w1, B_w2, B_w3, B_w4, c, w_mod,
):
    hbm = pl.BlockSpec(memory_space=pltpu.HBM)
    V = pltpu.VMEM
    out = pl.pallas_call(
        _kernel,
        out_shape=jax.ShapeDtypeStruct((S, D), BF16),
        in_specs=[hbm] * 14,
        out_specs=hbm,
        scratch_shapes=[
            V((4, D), BF16), V((1, D), BF16), V((1, D), BF16),
            V((2 * T, T), BF16), V((T, 2 * T), BF16),
            V((S, D), BF16), V((S, D), BF16), V((S, D), BF16), V((D, S), BF16),
            V((D, D), BF16), V((D, D), BF16), V((FF, D), BF16), V((FF, D), BF16),
            V((D, 6 * D), BF16), V((S, D), BF16),
            V((S + 8, D), F32), V((S, D), F32),
            V((NL, NB, 2 * T, 128), F32), V((NL, NB, 2 * T, 128), F32),
            V((NL, NB, 2 * T, 128), BF16),
            V((S + 16, D), F32), V((S, D), F32), V((S, D), F32),
            pltpu.SemaphoreType.DMA((14,)), pltpu.SemaphoreType.DMA((NC,)),
        ],
        compiler_params=pltpu.CompilerParams(vmem_limit_bytes=110 * 1024 * 1024),
    )(A_q[0], A_k[0], A_v[0], A_shift_k.T, A_ssm_k, A_ssm_D.reshape(1, D),
      B_w1, B_w2, B_w3.T, B_w4, c, w_mod,
      jnp.asarray(_FWD, BF16), jnp.asarray(_INV, BF16))
    return out[None]
```
